```python
import jax
import jax.numpy as jnp

def _softmax(x, axis=-1):
    return jax.nn.softmax(x, axis=axis)
def _gelu(x):
    return jax.nn.gelu(x, approximate=True)
def _silu(x):
    return jax.nn.silu(x)
def _sigmoid(x):
    return jax.nn.sigmoid(x)
def _layernorm(x, axis=-1, eps=1e-5):
    m = jnp.mean(x, axis=axis, keepdims=True)
    v = jnp.var(x, axis=axis, keepdims=True)
    return (x - m) / jnp.sqrt(v + eps)
def _scatter_add(tgt, idx, src, axis=0):
    return tgt.at[idx].add(src)
def _segment_sum(src, seg, n):
    return jax.ops.segment_sum(src, seg, n)
class _Rng:
    def __init__(self, key):
        self._k = key
    def _next(self):
        self._k, sub = jax.random.split(self._k)
        return sub
    def normal(self, shape):
        return jax.random.normal(self._next(), shape, dtype=jnp.bfloat16)
    def randint(self, lo, hi, shape):
        return jax.random.randint(self._next(), shape, lo, hi, dtype=jnp.int32)
    def uniform(self, shape, lo=0.0, hi=1.0):
        return jax.random.uniform(self._next(), shape, jnp.bfloat16, lo, hi)
    def permutation(self, n):
        return jax.random.permutation(self._next(), n)


kernel_name = 'concat_heads__mha_block_cached__compressed_kv_cla__decode'

def setup_inputs():
    _rng = _Rng(jax.random.key(int.from_bytes(__import__("os").urandom(4), "little")))
    _w = (lambda a: (lambda t: t.astype(jnp.bfloat16) if jnp.issubdtype(t.dtype, jnp.floating) else t)(jnp.asarray(a)))
    def _A_setup():
        B, Sq, D = 4, 1, 576
        H, Sk, Dh = 32, 4096, 128
        return {
            "x": _w((lambda *s: _rng.normal(s) * 0.05)(B, Sq, D)),
            "k_cache": _w((lambda *s: _rng.normal(s) * 0.05)(B, H, Sk, Dh)),
            "v_cache": _w((lambda *s: _rng.normal(s) * 0.05)(B, H, Sk, Dh)),
            "wq": _w((lambda *s: _rng.normal(s) * 0.05)(D, H * Dh) * (D ** -0.5)),
            "wo": _w((lambda *s: _rng.normal(s) * 0.05)(H * Dh, D) * ((H * Dh) ** -0.5)),
        }
    _A_in = _A_setup()

    def _B_setup():
        B, H, Sq, Sk, D, M = 4, 32, 1, 4096, 128, 576
        Dc = 4 * D
        return {
            "x": _w((lambda *s: _rng.normal(s) * 0.05)(B, Sq, M)),
            "c_kv": _w((lambda *s: _rng.normal(s) * 0.05)(B, Sk, Dc)),
            "w_q": _w((lambda *s: _rng.normal(s) * 0.05)(M, H, D) * (M ** -0.5)),
            "w_uk": _w((lambda *s: _rng.normal(s) * 0.05)(Dc, H, D) * (Dc ** -0.5)),
            "w_uv": _w((lambda *s: _rng.normal(s) * 0.05)(Dc, H, D) * (Dc ** -0.5)),
            "w_o": _w((lambda *s: _rng.normal(s) * 0.05)(H, D, M) * ((H * D) ** -0.5)),
        }
    _B_in = _B_setup()

    return {
        "A_x": _A_in["x"],
        "A_k_cache": _A_in["k_cache"],
        "A_v_cache": _A_in["v_cache"],
        "A_wq": _A_in["wq"],
        "A_wo": _A_in["wo"],
        "B_x": _B_in["x"],
        "B_c_kv": _B_in["c_kv"],
        "B_w_q": _B_in["w_q"],
        "B_w_uk": _B_in["w_uk"],
        "B_w_uv": _B_in["w_uv"],
        "B_w_o": _B_in["w_o"],
    }

def reference(A_x, A_k_cache, A_v_cache, A_wq, A_wo, B_x, B_c_kv, B_w_q, B_w_uk, B_w_uv, B_w_o):
    def _A_ref(x, k_cache, v_cache, wq, wo):
        B, Sq, D = x.shape
        H, Dh = 32, 128
        q = (lambda x, *d: x.transpose(*d))((x @ wq).reshape(B, Sq, H, Dh), 0, 2, 1, 3)
        scores = jnp.einsum("bhqd,bhkd->bhqk", q, k_cache) * (Dh ** -0.5)
        p = _softmax(scores, axis=-1)
        o = jnp.einsum("bhqk,bhkd->bhqd", p, v_cache)
        return (lambda x, *d: x.transpose(*d))(o, 0, 2, 1, 3).reshape(B, Sq, H * Dh) @ wo

    def _B_ref(x, c_kv, w_q, w_uk, w_uv, w_o):
        B, Sq, M = x.shape[0], x.shape[1], x.shape[2]
        Sk = c_kv.shape[1]
        H, D = w_q.shape[1], w_q.shape[2]
        q = jnp.einsum("bqm,mhd->bhqd", x, w_q)
        k = jnp.einsum("bkc,chd->bhkd", c_kv, w_uk)
        v = jnp.einsum("bkc,chd->bhkd", c_kv, w_uv)
        scores = jnp.einsum("bhqd,bhkd->bhqk", q, k) * (D ** -0.5)
        off = Sk - Sq
        qi = jnp.arange(Sq)[:, None]
        kj = jnp.arange(Sk)[None, :]
        cmask = kj <= (qi + off)
        scores = jnp.where(cmask[None, None], scores, -1e9)
        p = _softmax(scores, axis=-1)
        ctx = jnp.einsum("bhqk,bhkd->bhqd", p, v)
        return jnp.einsum("bhqd,hdm->bqm", ctx, w_o)

    a = _A_ref(A_x, A_k_cache, A_v_cache, A_wq, A_wo)
    b = _B_ref(B_x, B_c_kv, B_w_q, B_w_uk, B_w_uv, B_w_o)
    return jnp.concatenate([a, b], axis=-1)
```

```python
import jax
import jax.numpy as jnp
from jax import lax
import jax.experimental.pallas as pl
import jax.experimental.pallas.tpu as pltpu

_BF16 = jnp.bfloat16
_F32 = jnp.float32
_NT = (((1,), (1,)), ((), ()))

_DESC_BYTES = 32 * 1024
_LANES = 128
_RING = 4
_AHEAD = 2


def _dot(a, b):
    return jnp.dot(a, b, preferred_element_type=_F32)


def _dot_nt(a, b):
    return lax.dot_general(a, b, _NT, preferred_element_type=_F32)


class _Stream:
    def __init__(self, src, dst, sem, lo, rows):
        self.src, self.dst, self.sem, self.lo, self.rows = src, dst, sem, lo, rows
        width = src.shape[1]
        self.dcols = min(width, _DESC_BYTES // (8 * 2))
        self.drows = _DESC_BYTES // (self.dcols * 2)
        self.per_row = width // self.dcols
        self.count = rows // self.drows * self.per_row

    def start(self, group, size, k, priority):
        assert size % self.per_row == 0
        row = self.lo + (group * (size // self.per_row) + k // self.per_row) * self.drows
        if not isinstance(row, int):
            row = pl.multiple_of(row, self.drows)
        idx = (pl.ds(row, self.drows),)
        if self.per_row > 1:
            idx += (pl.ds(k % self.per_row * self.dcols, self.dcols),)
        pltpu.make_async_copy(self.src.at[idx], self.dst.at[idx], self.sem).start(
            priority=priority)

    def wait(self):
        full = self.dst.at[pl.ds(self.lo, self.rows)]
        pltpu.make_async_copy(full, full, self.sem).wait()


def _issue(unit, size=4):
    first, second = unit
    assert first.count == second.count and first.count % size == 0

    def body(g, carry):
        for k in range(size):
            first.start(g, size, k, 0)
            second.start(g, size, k, 1)
        return carry

    lax.fori_loop(0, first.count // size, body, 0)


def _wait(unit):
    for stream in unit:
        stream.wait()


def _kernel(ax_hbm, k_hbm, v_hbm, awq_hbm, awo_hbm, bx_hbm, c_hbm, bwq_hbm,
            wuk_hbm, wuv_hbm, bwo_hbm, out_ref,
            ax, bx, kbuf, vbuf, awq, awo, c, bwq, wuk, wuv, bwo,
            expand, qa, oa, prob, xsems, kvsems, sems):
    batch, model = ax.shape
    heads, _, dim = qa.shape
    seq = kbuf.shape[1]
    latent = c.shape[1]
    rows = batch * heads
    steps = batch * heads
    scale = dim ** -0.5
    m_blocks = [(lo, min(_LANES, model - lo)) for lo in range(0, model, _LANES)]
    c_blocks = list(range(0, latent, _LANES))

    next_sem = iter(range(sems.shape[0]))

    def unit(src0, dst0, lo0, n0, src1, dst1, lo1, n1):
        return (_Stream(src0, dst0, sems.at[next(next_sem)], lo0, n0),
                _Stream(src1, dst1, sems.at[next(next_sem)], lo1, n1))

    def kv_unit(i):
        slot = i % _RING
        return (_Stream(k_hbm.at[i], kbuf.at[slot], kvsems.at[slot], 0, seq),
                _Stream(v_hbm.at[i], vbuf.at[slot], kvsems.at[_RING + slot], 0, seq))

    wq_units = [unit(awq_hbm, awq, lo, n, bwq_hbm, bwq, lo * heads, n * heads)
                for lo, n in m_blocks]
    wu_units = [unit(wuk_hbm, wuk, lo * heads, _LANES * heads,
                     wuv_hbm, wuv, lo * heads, _LANES * heads) for lo in c_blocks]
    quarter = seq // 4
    c_units = [unit(c_hbm, c, b * seq + j * quarter, quarter,
                    c_hbm, c, b * seq + (j + 2) * quarter, quarter)
               for b in range(batch) for j in range(2)]
    wo_units = [unit(awo_hbm, awo, lo, n, bwo_hbm, bwo, lo * heads, n * heads)
                for lo, n in m_blocks]

    pending = iter(wq_units + wu_units + c_units + [kv_unit(i) for i in range(_RING)])

    def issue_next():
        _issue(next(pending))

    x_copies = [pltpu.make_async_copy(ax_hbm, ax, xsems.at[0]),
                pltpu.make_async_copy(bx_hbm, bx, xsems.at[1])]
    for copy in x_copies:
        copy.start()
    issue_next()

    shape = expand.shape
    expand[...] = jnp.where(
        lax.broadcasted_iota(jnp.int32, shape, 1) // heads
        == lax.broadcasted_iota(jnp.int32, shape, 0), 1.0, 0.0).astype(_BF16)
    oa[...] = jnp.zeros(oa.shape, _F32)

    def own_head(a):
        own = (lax.broadcasted_iota(jnp.int32, a.shape, 0) % heads
               == lax.broadcasted_iota(jnp.int32, a.shape, 1) % heads)
        return jnp.where(own, a, 0.0).astype(_BF16)

    def per_head_matmul(a, w):
        n = a.shape[1]
        return _dot(own_head(_dot(a, expand[:n, :n * heads])), w)

    for _ in range(_AHEAD - 1):
        issue_next()
    for copy in x_copies:
        copy.wait()
    xa = ax[...].astype(_F32)
    xa = jnp.concatenate([xa, jnp.zeros((8 - batch, model), _F32)], axis=0).astype(_BF16)
    xb = bx[...].astype(_F32)
    xb = jnp.concatenate(
        [jnp.broadcast_to(xb[b:b + 1], (heads, model)) for b in range(batch)],
        axis=0).astype(_BF16)

    q_a = jnp.zeros((8, heads * dim), _F32)
    q_b = jnp.zeros((rows, dim), _F32)
    for (lo, n), u in zip(m_blocks, wq_units):
        _wait(u)
        issue_next()
        q_a += _dot(xa[:, lo:lo + n], awq[lo:lo + n])
        q_b += per_head_matmul(xb[:, lo:lo + n], bwq[lo * heads:(lo + n) * heads])
    for h in range(heads):
        qa[h] = q_a[:, h * dim:(h + 1) * dim]
    q_b = q_b.astype(_BF16)

    q_lat = []
    for lo, u in zip(c_blocks, wu_units):
        _wait(u)
        issue_next()
        every = _dot_nt(q_b, wuk[lo * heads:(lo + _LANES) * heads])
        q_lat.append(_dot_nt(own_head(every), expand[...]).astype(_BF16))
    q_lat = jnp.concatenate(q_lat, axis=1)

    issue_next()
    ctx_lat = []
    for b in range(batch):
        _wait(c_units[2 * b])
        _wait(c_units[2 * b + 1])
        issue_next()
        s = _dot_nt(q_lat[b * heads:(b + 1) * heads], c[b * seq:(b + 1) * seq]) * scale
        p = jnp.exp(s - jnp.max(s, axis=-1, keepdims=True))
        denom = jnp.sum(p, axis=-1, keepdims=True)
        prob[...] = p.astype(_BF16)
        issue_next()
        ctx_lat.append((_dot(prob[...], c[b * seq:(b + 1) * seq]) / denom).astype(_BF16))
    ctx_lat = jnp.concatenate(ctx_lat, axis=0)
    issue_next()
    assert next(pending, None) is None

    def attend(i):
        b, h, slot = i // heads, i % heads, i % _RING
        _wait(kv_unit(i))
        s = _dot_nt(qa[h].astype(_BF16), kbuf[slot]) * scale
        p = jnp.exp(s - jnp.max(s, axis=-1, keepdims=True))
        o = _dot(p.astype(_BF16), vbuf[slot]) / jnp.sum(p, axis=-1, keepdims=True)
        oa[h] = jnp.where(lax.broadcasted_iota(jnp.int32, o.shape, 0) == b, o, oa[h])

    def step(i, carry):
        attend(i)
        _issue(kv_unit(i + _RING))
        return carry

    ctx = jnp.zeros((rows, dim), _F32)
    for i, lo in enumerate(c_blocks):
        step(i, 0)
        ctx += per_head_matmul(ctx_lat[:, lo:lo + _LANES],
                               wuv[lo * heads:(lo + _LANES) * heads])
    dst = lax.broadcasted_iota(jnp.int32, (heads * 8, rows), 0)
    src = lax.broadcasted_iota(jnp.int32, (heads * 8, rows), 1)
    regroup = jnp.where(dst % 8 * heads + dst // 8 == src, 1.0, 0.0).astype(_BF16)
    ctx = _dot(regroup, ctx.astype(_BF16))

    lax.fori_loop(len(c_blocks), steps - _RING, step, 0)

    pending = iter(wo_units)
    for i in range(steps - _RING, steps):
        attend(i)
        if i % 2 == 0:
            issue_next()
    o_a = jnp.concatenate([oa[h] for h in range(heads)], axis=1).astype(_BF16)
    out_a = []
    out_b = jnp.zeros((8, model), _F32)
    done = 0
    for (lo, n), u in zip(m_blocks, wo_units):
        _wait(u)
        u = next(pending, None)
        if u is not None:
            _issue(u)
        out_a.append(_dot_nt(o_a, awo[lo:lo + n]))
        for h in range(done, (lo + n) * heads // model):
            out_b += _dot_nt(ctx[h * 8:(h + 1) * 8].astype(_BF16),
                             bwo[h * model:(h + 1) * model])
            done = h + 1
    out = jnp.concatenate(out_a + [out_b], axis=1)
    out_ref[...] = out[:batch].astype(out_ref.dtype)


@jax.jit
def pallas_concat_heads__mha_block_cached__compressed_kv_cla__decode_kernel(
    A_x: jax.Array,
    A_k_cache: jax.Array,
    A_v_cache: jax.Array,
    A_wq: jax.Array,
    A_wo: jax.Array,
    B_x: jax.Array,
    B_c_kv: jax.Array,
    B_w_q: jax.Array,
    B_w_uk: jax.Array,
    B_w_uv: jax.Array,
    B_w_o: jax.Array,
):
    batch, heads, seq, dim = A_k_cache.shape
    model = A_x.shape[-1]
    latent = B_c_kv.shape[-1]
    operands = (
        A_x.reshape(batch, model),
        A_k_cache.reshape(batch * heads, seq, dim),
        A_v_cache.reshape(batch * heads, seq, dim),
        A_wq,
        A_wo.T,
        B_x.reshape(batch, model),
        B_c_kv.reshape(batch * seq, latent),
        B_w_q.reshape(model * heads, dim),
        B_w_uk.reshape(latent * heads, dim),
        B_w_uv.reshape(latent * heads, dim),
        B_w_o.transpose(0, 2, 1).reshape(heads * model, dim),
    )
    resident = lambda i: pltpu.VMEM(operands[i].shape, _BF16)
    ring = pltpu.VMEM((_RING, seq, dim), _BF16)
    n_units = 2 * pl.cdiv(model, _LANES) + latent // _LANES + 2 * batch
    out = pl.pallas_call(
        _kernel,
        in_specs=[pl.BlockSpec(memory_space=pltpu.HBM)] * len(operands),
        out_shape=jax.ShapeDtypeStruct((batch, 2 * model), A_x.dtype),
        scratch_shapes=[
            resident(0), resident(5), ring, ring, resident(3), resident(4),
            resident(6), resident(7), resident(8), resident(9), resident(10),
            pltpu.VMEM((_LANES, _LANES * heads), _BF16),
            pltpu.VMEM((heads, 8, dim), _F32),
            pltpu.VMEM((heads, 8, dim), _F32),
            pltpu.VMEM((heads, seq), _BF16),
            pltpu.SemaphoreType.DMA((2,)),
            pltpu.SemaphoreType.DMA((2 * _RING,)),
            pltpu.SemaphoreType.DMA((2 * n_units,)),
        ],
        compiler_params=pltpu.CompilerParams(vmem_limit_bytes=100 * 1024 * 1024),
    )(*operands)
    return out.reshape(batch, 1, 2 * model)
```

```python
import jax
import jax.numpy as jnp
from jax import lax
import jax.experimental.pallas as pl
import jax.experimental.pallas.tpu as pltpu

_BF16 = jnp.bfloat16
_F32 = jnp.float32
_NT = (((1,), (1,)), ((), ()))

_LANES = 128
_AHEAD = 4
_GROUP = 8
_W_SEG = 64
_C_SEG = 1024
_O_STEP = 2


def _dot(a, b):
    return jnp.dot(a, b, preferred_element_type=_F32)


def _dot_nt(a, b):
    return lax.dot_general(a, b, _NT, preferred_element_type=_F32)


def _loop(n, body):
    lax.fori_loop(0, n, lambda i, carry: (body(i), carry)[1], 0)


def _block(i, n):
    return pl.ds(pl.multiple_of(i * n, n), n)


def _issue(unit, run_kib, parts):
    run = run_kib * 512

    def fetch(r):
        for k in range(parts):
            for priority, (src, dst, sem) in enumerate(unit):
                segments, _, width = src.shape
                lo, hi = k * segments // parts, (k + 1) * segments // parts
                if run >= 8 * width:
                    idx = (pl.ds(lo, hi - lo), _block(r, run // width))
                else:
                    across = 8 * width // run
                    idx = (pl.ds(lo, hi - lo), _block(lax.div(r, across), 8),
                           _block(lax.rem(r, across), run // 8))
                pltpu.make_async_copy(src.at[idx], dst.at[idx], sem).start(priority=priority)

    sizes = [src.shape[1] * src.shape[2] for src, _, _ in unit]
    assert sizes[0] == sizes[1] and sizes[0] % run == 0
    _loop(sizes[0] // run, fetch)


def _wait(unit):
    for _, dst, sem in unit:
        pltpu.make_async_copy(dst, dst, sem).wait()


def _own_block(a):
    n, w = a.shape[0], a.shape[1] // a.shape[0]
    row = lax.broadcasted_iota(jnp.int32, (n, w), 0)
    out = a[:, :w]
    for j in range(1, n):
        out = jnp.where(row == j, a[:, j * w:(j + 1) * w], out)
    return out


def _block_diagonal(a):
    row = lax.broadcasted_iota(jnp.int32, a.shape, 0)
    return jnp.concatenate(
        [jnp.where(row == j, a, 0.0) for j in range(a.shape[0])], axis=1).astype(_BF16)


def _softmax_step(s, max_ref, sum_ref):
    old_max = max_ref[...]
    new_max = jnp.maximum(old_max, jnp.max(s, axis=-1, keepdims=True))
    p = jnp.exp(s - new_max[:, :1])
    decay = jnp.exp(old_max - new_max)
    max_ref[...] = new_max
    sum_ref[...] = decay * sum_ref[...] + jnp.sum(p, axis=-1, keepdims=True)
    return p, decay


def _kernel(ax_hbm, k_hbm, v_hbm, awq_hbm, awo_hbm, bx_hbm, c_hbm, bwq_hbm,
            wuk_hbm, wuv_hbm, bwo_hbm, out_ref,
            ax, kbuf, vbuf, awq, awo, bx, c, bwq, wuk, wuv, bwo,
            xa, q_a, max_a, sum_a, ctx_a, out_a,
            expand, xb, q_b, q_lat, max_b, sum_b, ctx_lat, ctx_b, ctx_hb, out_b,
            x_sems, sems):
    batch, model = ax.shape
    heads, _, dim = bwo.shape
    keys = kbuf.shape[2]
    scale = dim ** -0.5
    pieces = _LANES // _W_SEG
    n_kv, n_wo = batch * heads, heads // (2 * _O_STEP)

    def unit(n, *copies):
        slot = lax.rem(n, _AHEAD)
        return [(*copy, sems.at[2 * slot + k]) for k, copy in enumerate(copies)]

    def halves(src, dst):
        cut = src.shape[0] // 2
        return [(src.at[part], dst.at[part])
                for part in (pl.ds(0, cut), pl.ds(cut, src.shape[0] - cut))]

    def kv_unit(i):
        idx = (_block(lax.div(i, _GROUP), _GROUP), _block(lax.rem(i, _GROUP), keys))
        slot = lax.rem(i, _AHEAD)
        return unit(i, (k_hbm.at[idx], kbuf.at[slot]), (v_hbm.at[idx], vbuf.at[slot]))

    def wo_unit(j):
        return unit(j, *[(bwo_hbm.at[part], bwo.at[part])
                         for part in (_block(j, _O_STEP), _block(n_wo + j, _O_STEP))])

    issue_kv = lambda i: _issue(kv_unit(i), 16, 4)
    issue_wo = lambda j: _issue(wo_unit(j), 16, 2)
    x_unit = [(ax_hbm, ax, x_sems.at[0]), (bx_hbm, bx, x_sems.at[1])]
    first_units = [
        (unit(0, (awq_hbm, awq), (bwq_hbm, bwq)), 8, 2),
        (unit(1, (wuk_hbm, wuk), (wuv_hbm, wuv)), 8, 2),
        (unit(2, *halves(awo_hbm, awo)), 8, 1),
        (unit(3, *halves(c_hbm, c)), 16, 4),
    ]
    assert len(first_units) == _AHEAD and n_kv % _AHEAD == 0

    for copy in x_unit:
        pltpu.make_async_copy(*copy).start()
    for first in first_units:
        _issue(*first)

    def build_expand(t):
        k, g = lax.div(t, _LANES // 16), lax.rem(t, _LANES // 16)
        shape = (16, expand.shape[2])
        col = lax.shift_right_logical(
            lax.broadcasted_iota(jnp.int32, shape, 1), heads.bit_length() - 1)
        row = lax.broadcasted_iota(jnp.int32, shape, 0) + (g * 16 - k * _W_SEG)
        expand[k, _block(g, 16)] = jnp.where(col == row, 1.0, 0.0).astype(_BF16)

    _loop(pieces * _LANES // 16, build_expand)
    for ref in (out_a, q_b, q_lat, sum_b, ctx_lat, ctx_b, out_b):
        ref[...] = jnp.zeros(ref.shape, _F32)
    max_b[...] = jnp.full(max_b.shape, -jnp.inf, _F32)

    _wait(x_unit)
    x = ax[...].astype(_F32)
    for b in range(batch):
        xa[b] = jnp.broadcast_to(x[b:b + 1], xa.shape[1:])
    x = jnp.concatenate(
        [bx[...].astype(_F32), jnp.zeros((batch, -model % _LANES), _F32)], axis=1)
    for b in range(batch):
        for i in range(xb.shape[0]):
            xb[i, b * heads:(b + 1) * heads] = jnp.broadcast_to(
                x[b:b + 1, i * _LANES:(i + 1) * _LANES], (heads, _LANES))

    for i, (first, _, _) in enumerate(first_units):
        _wait(first)
        issue_kv(i)

    def own_head(a):
        differ = (lax.broadcasted_iota(jnp.int32, a.shape, 0)
                  ^ lax.broadcasted_iota(jnp.int32, a.shape, 1)) & (heads - 1)
        return jnp.where(differ == 0, a, 0.0).astype(_BF16)

    def per_head_matmul(acc, a, w, t):
        spread = _dot(a[lax.div(t, pieces)].astype(_BF16), expand[lax.rem(t, pieces)])
        acc[...] += _dot(own_head(spread), w[t])

    def absorb(t):
        every = _dot_nt(q_b[...].astype(_BF16), wuk[t])
        q_lat[lax.div(t, pieces)] += _dot_nt(own_head(every), expand[lax.rem(t, pieces)])

    def attend_latent(t):
        rows = _block(lax.div(t, c.shape[0] // batch), heads)
        blocks = range(q_lat.shape[0])
        q = jnp.concatenate([q_lat[i, rows] for i in blocks], axis=1).astype(_BF16)
        p, decay = _softmax_step(_dot_nt(q, c[t]) * scale, max_b.at[rows], sum_b.at[rows])
        o = _dot(p.astype(_BF16), c[t])
        for i in blocks:
            ctx_lat[i, rows] = decay * ctx_lat[i, rows] + o[:, i * _LANES:(i + 1) * _LANES]

    def normalise(_):
        ctx_lat[...] = ctx_lat[...] / sum_b[...]

    def regroup(_):
        dst = lax.broadcasted_iota(jnp.int32, (heads * 8, batch * heads), 0)
        src = lax.broadcasted_iota(jnp.int32, (heads * 8, batch * heads), 1)
        move = jnp.where((dst & 7) * heads + (dst >> 3) == src, 1.0, 0.0)
        ctx_hb[...] = _dot(move.astype(_BF16), ctx_b[...].astype(_BF16))

    b_tasks = [
        (bwq.shape[0], lambda t: per_head_matmul(q_b, xb, bwq, t)),
        (wuk.shape[0], absorb),
        (c.shape[0], attend_latent),
        (1, normalise),
        (wuv.shape[0], lambda t: per_head_matmul(ctx_b, ctx_lat, wuv, t)),
        (1, regroup),
    ]

    def attend_cache(i):
        b, chunk, slot = lax.div(i, heads), lax.rem(i, _GROUP), lax.rem(i, _AHEAD)
        cols = _block(lax.div(lax.rem(i, heads), _GROUP), _GROUP * dim)

        @pl.when(chunk == 0)
        def _():
            w = awq[:, :, cols].reshape(model, _GROUP * dim)
            q_a[...] = _own_block(_dot(xa[b].astype(_BF16), w))
            max_a[...] = jnp.full(max_a.shape, -jnp.inf, _F32)
            sum_a[...] = jnp.zeros(sum_a.shape, _F32)
            ctx_a[...] = jnp.zeros(ctx_a.shape, _F32)

        s = _dot_nt(q_a[...].astype(_BF16), kbuf[slot].reshape(_GROUP * keys, dim))
        p, decay = _softmax_step(_own_block(s) * scale, max_a, sum_a)
        ctx_a[...] = decay * ctx_a[...] + _dot(
            _block_diagonal(p), vbuf[slot].reshape(_GROUP * keys, dim))

        @pl.when(chunk == _GROUP - 1)
        def _():
            w = awo[:, :, cols].reshape(model, _GROUP * dim)
            out_a[b] += _dot_nt(_block_diagonal(ctx_a[...] / sum_a[...]), w)

    def step(i):
        _wait(kv_unit(i))
        attend_cache(i)
        pl.when(i + _AHEAD < n_kv)(lambda: issue_kv(i + _AHEAD))
        pl.when(i + _AHEAD >= n_kv)(lambda: issue_wo(i + _AHEAD - n_kv))
        t, first = jnp.where(lax.rem(i, 2) == 1, lax.div(i, 2), -1), 0
        for count, task in b_tasks:
            pl.when((t >= first) & (t < first + count))(lambda: task(t - first))
            first += count
        assert 2 * first <= n_kv

    _loop(n_kv, step)
    a = jnp.concatenate(
        [jnp.sum(out_a[b], axis=0, keepdims=True) for b in range(batch)], axis=0)

    def project(j):
        _wait(wo_unit(j))
        pl.when(j + _AHEAD < n_wo)(lambda: issue_wo(j + _AHEAD))
        out_b[...] += sum(
            _dot_nt(ctx_hb[_block(h, 8)].astype(_BF16), bwo[h])
            for half in (j, n_wo + j) for k in range(_O_STEP)
            for h in [half * _O_STEP + k])

    _loop(n_wo, project)
    out_ref[...] = jnp.concatenate([a, out_b[:batch]], axis=1).astype(out_ref.dtype)


@jax.jit
def pallas_concat_heads__mha_block_cached__compressed_kv_cla__decode_kernel(
    A_x: jax.Array,
    A_k_cache: jax.Array,
    A_v_cache: jax.Array,
    A_wq: jax.Array,
    A_wo: jax.Array,
    B_x: jax.Array,
    B_c_kv: jax.Array,
    B_w_q: jax.Array,
    B_w_uk: jax.Array,
    B_w_uv: jax.Array,
    B_w_o: jax.Array,
):
    batch, heads, seq, dim = A_k_cache.shape
    model = A_x.shape[-1]
    latent = B_c_kv.shape[-1]
    operands = (
        A_x.reshape(batch, model),
        A_k_cache.reshape(batch * heads, seq, dim),
        A_v_cache.reshape(batch * heads, seq, dim),
        A_wq.reshape(-1, _W_SEG, heads * dim),
        A_wo.T.reshape(-1, _W_SEG, heads * dim),
        B_x.reshape(batch, model),
        B_c_kv.reshape(-1, _C_SEG, latent),
        B_w_q.reshape(-1, _W_SEG * heads, dim),
        B_w_uk.reshape(-1, _W_SEG * heads, dim),
        B_w_uv.reshape(-1, _W_SEG * heads, dim),
        B_w_o.transpose(0, 2, 1),
    )
    buffers = [pltpu.VMEM(operand.shape, _BF16) for operand in operands]
    buffers[1:3] = [pltpu.VMEM((_AHEAD, _GROUP, seq // _GROUP, dim), _BF16)] * 2
    f32 = lambda *shape: pltpu.VMEM(shape, _F32)
    rows = batch * heads
    out = pl.pallas_call(
        _kernel,
        in_specs=[pl.BlockSpec(memory_space=pltpu.HBM)] * len(operands),
        out_shape=jax.ShapeDtypeStruct((batch, 2 * model), A_x.dtype),
        scratch_shapes=[
            *buffers,
            f32(batch, _GROUP, model), *[f32(_GROUP, dim)] * 4, f32(batch, _GROUP, model),
            pltpu.VMEM((_LANES // _W_SEG, _LANES, _W_SEG * heads), _BF16),
            f32(pl.cdiv(model, _LANES), rows, _LANES), f32(rows, dim),
            f32(latent // _LANES, rows, _LANES), f32(rows, _LANES), f32(rows, _LANES),
            f32(latent // _LANES, rows, _LANES), f32(rows, dim), f32(heads * 8, dim),
            f32(8, model),
            pltpu.SemaphoreType.DMA((2,)), pltpu.SemaphoreType.DMA((2 * _AHEAD,)),
        ],
        compiler_params=pltpu.CompilerParams(vmem_limit_bytes=100 * 1024 * 1024),
    )(*operands)
    return out.reshape(batch, 1, 2 * model)
```
